```python
import jax
import jax.numpy as jnp

def _softmax(x, axis=-1):
    return jax.nn.softmax(x, axis=axis)
def _gelu(x):
    return jax.nn.gelu(x, approximate=True)
def _silu(x):
    return jax.nn.silu(x)
def _sigmoid(x):
    return jax.nn.sigmoid(x)
def _layernorm(x, axis=-1, eps=1e-5):
    m = jnp.mean(x, axis=axis, keepdims=True)
    v = jnp.var(x, axis=axis, keepdims=True)
    return (x - m) / jnp.sqrt(v + eps)
def _scatter_add(tgt, idx, src, axis=0):
    return tgt.at[idx].add(src)
def _segment_sum(src, seg, n):
    return jax.ops.segment_sum(src, seg, n)
class _Rng:
    def __init__(self, key):
        self._k = key
    def _next(self):
        self._k, sub = jax.random.split(self._k)
        return sub
    def normal(self, shape):
        return jax.random.normal(self._next(), shape, dtype=jnp.bfloat16)
    def randint(self, lo, hi, shape):
        return jax.random.randint(self._next(), shape, lo, hi, dtype=jnp.int32)
    def uniform(self, shape, lo=0.0, hi=1.0):
        return jax.random.uniform(self._next(), shape, jnp.bfloat16, lo, hi)
    def permutation(self, n):
        return jax.random.permutation(self._next(), n)


kernel_name = 'interleave_layers__sliding_block_cached__dense_activation_gelu__decode'

def _fwd_setup_inputs():
    _rng = _Rng(jax.random.key(int.from_bytes(__import__("os").urandom(4), "little")))
    _w = (lambda a: (lambda t: t.astype(jnp.bfloat16) if jnp.issubdtype(t.dtype, jnp.floating) else t)(jnp.asarray(a)))
    def _A_setup():
        B, Sq, D = 2, 1, 512
        Hq, Hkv, Sk, Dh = 32, 8, 32768, 128
        assert Hq % Hkv == 0, (Hq, Hkv)
        return {
            "x": _w((lambda *s: _rng.normal(s) * 0.05)(B, Sq, D)),
            "k_cache": _w((lambda *s: _rng.normal(s) * 0.05)(B, Hkv, Sk, Dh)),
            "v_cache": _w((lambda *s: _rng.normal(s) * 0.05)(B, Hkv, Sk, Dh)),
            "wq": _w((lambda *s: _rng.normal(s) * 0.05)(D, Hq * Dh) * (D ** -0.5)),
            "wo": _w((lambda *s: _rng.normal(s) * 0.05)(Hq * Dh, D) * ((Hq * Dh) ** -0.5)),
        }
    _A_in = _A_setup()

    def _B_setup():
        B, S, D, F = 2, 1, 512, 1792
        return {
            "x": _w((lambda *s: _rng.normal(s) * 0.05)(B, S, D)),
            "w1": _w((lambda *s: _rng.normal(s) * 0.05)(D, F) * (D ** -0.5)),
            "b1": _w((lambda *s: _rng.normal(s) * 0.05)(F) * 0.01),
            "w2": _w((lambda *s: _rng.normal(s) * 0.05)(F, D) * (F ** -0.5)),
            "b2": _w((lambda *s: _rng.normal(s) * 0.05)(D) * 0.01),
        }
    _B_in = _B_setup()

    return {
        "A_x": _A_in["x"],
        "A_k_cache": _A_in["k_cache"],
        "A_v_cache": _A_in["v_cache"],
        "A_wq": _A_in["wq"],
        "A_wo": _A_in["wo"],
        "B_x": _B_in["x"],
        "B_w1": _B_in["w1"],
        "B_b1": _B_in["b1"],
        "B_w2": _B_in["w2"],
        "B_b2": _B_in["b2"],
    }

def _fwd_reference(A_x, A_k_cache, A_v_cache, A_wq, A_wo, B_x, B_w1, B_b1, B_w2, B_b2):
    def _A_ref(x, k_cache, v_cache, wq, wo):
        B, Sq, D = x.shape
        Hq, Dh = 32, 128
        Hkv, Sk = k_cache.shape[1], k_cache.shape[2]
        W = min(4096, max(256, Sk // 4))
        rep = Hq // Hkv
        q = (lambda x, *d: x.transpose(*d))((x @ wq).reshape(B, Sq, Hq, Dh), 0, 2, 1, 3)
        k = jnp.repeat(k_cache[:, :, Sk - W:, :], rep, axis=1)
        v = jnp.repeat(v_cache[:, :, Sk - W:, :], rep, axis=1)
        scores = jnp.einsum("bhqd,bhkd->bhqk", q, k) * (Dh ** -0.5)
        p = _softmax(scores, axis=-1)
        o = jnp.einsum("bhqk,bhkd->bhqd", p, v)
        return (lambda x, *d: x.transpose(*d))(o, 0, 2, 1, 3).reshape(B, Sq, Hq * Dh) @ wo

    def _B_ref(x, w1, b1, w2, b2):
        h = jnp.einsum("bsd,df->bsf", x, w1) + b1
        h = _gelu(h)
        return jnp.einsum("bsf,fd->bsd", h, w2) + b2

    x = A_x
    x = x + _A_ref(_layernorm(x, axis=-1), A_k_cache, A_v_cache, A_wq, A_wo)
    x = x + _B_ref(_layernorm(x, axis=-1), B_w1, B_b1, B_w2, B_b2)
    x = x + _A_ref(_layernorm(x, axis=-1), A_k_cache, A_v_cache, A_wq, A_wo)
    x = x + _B_ref(_layernorm(x, axis=-1), B_w1, B_b1, B_w2, B_b2)
    return x


def setup_inputs():
    _inp = _fwd_setup_inputs()
    _gk = jax.random.fold_in(jax.random.key(int.from_bytes(__import__("os").urandom(4), "little")), 2**31 - 1)
    _shapes = [[2, 1, 512]]
    _dtypes = ['bfloat16']
    _gks = jax.random.split(_gk, len(_shapes))
    _gs = [jax.random.normal(k, s, dtype=jnp.dtype(d)) * 0.05 for k, s, d in zip(_gks, _shapes, _dtypes)]
    _inp["grad_out"] = _gs[0]
    return _inp

def reference(A_x, A_k_cache, A_v_cache, A_wq, A_wo, B_w1, B_b1, B_w2, B_b2, B_x, grad_out):
    _const = dict(B_x=B_x)
    def _f(*_d):
        return _fwd_reference(**{'A_x': _d[0], 'A_k_cache': _d[1], 'A_v_cache': _d[2], 'A_wq': _d[3], 'A_wo': _d[4], 'B_w1': _d[5], 'B_b1': _d[6], 'B_w2': _d[7], 'B_b2': _d[8], **_const})
    _out, _vjp = jax.vjp(_f, A_x, A_k_cache, A_v_cache, A_wq, A_wo, B_w1, B_b1, B_w2, B_b2)
    _grads = _vjp(grad_out)
    _out0 = jnp.asarray(_out)
    return (_out0, *[jnp.asarray(_g) for _g in _grads])
```

```python
import functools
import math

import jax
import jax.numpy as jnp
import jax.experimental.pallas as pl
import jax.experimental.pallas.tpu as pltpu

_F32 = jnp.float32
_BF16 = jnp.bfloat16
_EPS = 1e-5
_GELU_C = math.sqrt(2.0 / math.pi)
_GELU_A = 0.044715

_NT = (((1,), (1,)), ((), ()))
_TN = (((0,), (0,)), ((), ()))


def _dot(a, b):
    return jnp.dot(a, b, preferred_element_type=_F32)


def _dot_nt(a, b):
    return jax.lax.dot_general(a, b, _NT, preferred_element_type=_F32)


def _dot_tn(a, b):
    return jax.lax.dot_general(a, b, _TN, preferred_element_type=_F32)


def _ln_fwd(x):
    m = jnp.mean(x, axis=-1, keepdims=True)
    xc = x - m
    v = jnp.mean(xc * xc, axis=-1, keepdims=True)
    rstd = 1.0 / jnp.sqrt(v + _EPS)
    return xc * rstd, rstd


def _ln_bwd(dn, n, rstd):
    return (dn - jnp.mean(dn, axis=-1, keepdims=True)
            - n * jnp.mean(dn * n, axis=-1, keepdims=True)) * rstd


def _gelu_fwd(h):
    t = jnp.tanh(_GELU_C * (h + _GELU_A * h * h * h))
    return 0.5 * h * (1.0 + t), t


def _gelu_grad(h, t):
    return 0.5 * (1.0 + t) + 0.5 * h * (1.0 - t * t) * _GELU_C * (1.0 + 3.0 * _GELU_A * h * h)


def _make_kernel(B, D, Hq, Hkv, Sk, Dh, W, F, zrows):
    rep = Hq // Hkv
    G = B * Hkv
    scale = Dh ** -0.5
    nz = Sk - W
    assert 2 * rep == 8 and nz % zrows == 0

    def kernel(x_ref, go_ref, b1_ref, b2_ref,
               k_hbm, v_hbm, wq_hbm, wo_hbm, w1_hbm, w2_hbm,
               out_ref, gx_ref, db1_ref, db2_ref,
               dk_hbm, dv_hbm, dwq_hbm, dwo_hbm, dw1_hbm, dw2_hbm,
               kbuf, vbuf, wq, wo, w1, w2, gwq, gwo, gw1, gw2, zbuf,
               q_scr, do_scr, a_scr, p_scr, flat_scr,
               ksem, vsem, wsem, zsem, osem):
        def k_in(i):
            return pltpu.make_async_copy(
                k_hbm.at[i // Hkv, i % Hkv, pl.ds(nz, W), :], kbuf.at[i], ksem.at[i])

        def v_in(i):
            return pltpu.make_async_copy(
                v_hbm.at[i // Hkv, i % Hkv, pl.ds(nz, W), :], vbuf.at[i], vsem.at[i])

        def k_out(i):
            return pltpu.make_async_copy(
                kbuf.at[i], dk_hbm.at[i // Hkv, i % Hkv, pl.ds(nz, W), :], ksem.at[i])

        def v_out(i):
            return pltpu.make_async_copy(
                vbuf.at[i], dv_hbm.at[i // Hkv, i % Hkv, pl.ds(nz, W), :], vsem.at[i])

        w_in = [pltpu.make_async_copy(s, d, wsem.at[j]) for j, (s, d) in enumerate(
            ((wq_hbm, wq), (wo_hbm, wo), (w1_hbm, w1), (w2_hbm, w2)))]
        w_out = [pltpu.make_async_copy(s, d, osem.at[j]) for j, (s, d) in enumerate(
            ((gwq, dwq_hbm), (gwo, dwo_hbm), (gw1, dw1_hbm), (gw2, dw2_hbm)))]

        w_in[0].start()
        for i in range(G):
            k_in(i).start()
            v_in(i).start()
        for c in w_in[1:]:
            c.start()

        zbuf[...] = jnp.zeros(zbuf.shape, zbuf.dtype)
        zfill = []
        for i in range(G):
            for o_hbm in (dk_hbm, dv_hbm):
                for c in range(nz // zrows):
                    cp = pltpu.make_async_copy(
                        zbuf, o_hbm.at[i // Hkv, i % Hkv, pl.ds(c * zrows, zrows), :], zsem.at[0])
                    cp.start()
                    zfill.append(cp)

        q_scr[...] = jnp.zeros(q_scr.shape, _F32)
        do_scr[...] = jnp.zeros(do_scr.shape, _F32)

        def scatter_heads(dst, flat, layer):
            for b in range(B):
                for h in range(Hq):
                    dst[b * Hkv + h // rep, pl.ds(layer * rep + h % rep, 1), :] = (
                        flat[b:b + 1, h * Dh:(h + 1) * Dh])

        def gather_heads(src, layer):
            for b in range(B):
                for h in range(Hq):
                    flat_scr[pl.ds(b, 1), pl.ds(h * Dh, Dh)] = (
                        src[b * Hkv + h // rep, pl.ds(layer * rep + h % rep, 1), :])
            return flat_scr[...]

        def attn_fwd(first):
            def body(i, carry):
                if first:
                    k_in(i).wait()
                s = _dot_nt(q_scr[i].astype(_BF16), kbuf[i]) * scale
                m = jnp.max(s, axis=-1, keepdims=True)
                e = jnp.exp(s - m)
                p = e / jnp.sum(e, axis=-1, keepdims=True)
                p_scr[i] = p
                if first:
                    v_in(i).wait()
                a_scr[i] = _dot(p.astype(_BF16), vbuf[i])
                return carry
            jax.lax.fori_loop(0, G, body, 0)

        def attn_bwd(last):
            def body(i, carry):
                do = do_scr[i].astype(_BF16)
                p = p_scr[i]
                dp = _dot_nt(do, vbuf[i])
                ds = (p * (dp - jnp.sum(dp * p, axis=-1, keepdims=True)) * scale).astype(_BF16)
                a_scr[i] = _dot(ds, kbuf[i])
                if last:
                    kbuf[i] = _dot_tn(ds, q_scr[i].astype(_BF16)).astype(_BF16)
                    k_out(i).start()
                    vbuf[i] = _dot_tn(p.astype(_BF16), do).astype(_BF16)
                    v_out(i).start()
                return carry
            jax.lax.fori_loop(0, G, body, 0)

        b1 = b1_ref[...].astype(_F32)
        b2 = b2_ref[...].astype(_F32)

        x = x_ref[...].astype(_F32)
        saved = []
        for layer in range(2):
            n_a, r_a = _ln_fwd(x)
            if layer == 0:
                w_in[0].wait()
            q = _dot(n_a.astype(_BF16), wq[...])
            scatter_heads(q_scr, q, layer)
            attn_fwd(layer == 0)
            o = gather_heads(a_scr, layer)
            if layer == 0:
                w_in[1].wait()
            x = x + _dot(o.astype(_BF16), wo[...])
            n_m, r_m = _ln_fwd(x)
            if layer == 0:
                w_in[2].wait()
            h = _dot(n_m.astype(_BF16), w1[...]) + b1
            g, t = _gelu_fwd(h)
            if layer == 0:
                w_in[3].wait()
            x = x + _dot(g.astype(_BF16), w2[...]) + b2
            saved.append((n_a, r_a, o, n_m, r_m, h, g, t))
        out_ref[...] = x.astype(out_ref.dtype)

        dx = go_ref[...].astype(_F32)
        grads = [None, None]
        for layer in (1, 0):
            n_a, r_a, o, n_m, r_m, h, g, t = saved[layer]
            dm = dx
            dg = _dot_nt(dm.astype(_BF16), w2[...])
            dh = dg * _gelu_grad(h, t)
            dn = _dot_nt(dh.astype(_BF16), w1[...])
            dx = dx + _ln_bwd(dn, n_m, r_m)
            da = dx
            do = _dot_nt(da.astype(_BF16), wo[...])
            scatter_heads(do_scr, do, layer)
            attn_bwd(layer == 0)
            dq = gather_heads(a_scr, layer)
            dn = _dot_nt(dq.astype(_BF16), wq[...])
            dx = dx + _ln_bwd(dn, n_a, r_a)
            grads[layer] = (dm, dh, da, dq)
        gx_ref[...] = dx.astype(gx_ref.dtype)

        def stack(a0, a1):
            return jnp.concatenate([a0, a1], axis=0).astype(_BF16)

        s0, s1 = saved
        g0, g1 = grads
        gwq[...] = _dot_tn(stack(s0[0], s1[0]), stack(g0[3], g1[3])).astype(_BF16)
        w_out[0].start()
        gwo[...] = _dot_tn(stack(s0[2], s1[2]), stack(g0[2], g1[2])).astype(_BF16)
        w_out[1].start()
        gw1[...] = _dot_tn(stack(s0[3], s1[3]), stack(g0[1], g1[1])).astype(_BF16)
        w_out[2].start()
        gw2[...] = _dot_tn(stack(s0[6], s1[6]), stack(g0[0], g1[0])).astype(_BF16)
        w_out[3].start()
        db1_ref[...] = jnp.sum(g0[1] + g1[1], axis=0, keepdims=True).astype(db1_ref.dtype)
        db2_ref[...] = jnp.sum(g0[0] + g1[0], axis=0, keepdims=True).astype(db2_ref.dtype)

        for cp in zfill:
            cp.wait()
        for i in range(G):
            k_out(i).wait()
            v_out(i).wait()
        for c in w_out:
            c.wait()

    return kernel


@jax.jit
def pallas_interleave_layers__sliding_block_cached__dense_activation_gelu__decode_kernel(
    A_x: jax.Array,
    A_k_cache: jax.Array,
    A_v_cache: jax.Array,
    A_wq: jax.Array,
    A_wo: jax.Array,
    B_x: jax.Array,
    B_w1: jax.Array,
    B_b1: jax.Array,
    B_w2: jax.Array,
    B_b2: jax.Array,
    grad_out: jax.Array,
):
    B, Sq, D = A_x.shape
    assert Sq == 1
    Hq, Dh = 32, 128
    Hkv, Sk = A_k_cache.shape[1], A_k_cache.shape[2]
    W = min(4096, max(256, Sk // 4))
    F = B_w1.shape[1]
    G = B * Hkv
    zrows = 4096

    kernel = _make_kernel(B, D, Hq, Hkv, Sk, Dh, W, F, zrows)

    vmem = pl.BlockSpec(memory_space=pltpu.VMEM)
    hbm = pl.BlockSpec(memory_space=pl.ANY)
    dt = A_x.dtype
    out_shape = (
        jax.ShapeDtypeStruct((B, D), dt),
        jax.ShapeDtypeStruct((B, D), dt),
        jax.ShapeDtypeStruct((1, F), dt),
        jax.ShapeDtypeStruct((1, D), dt),
        jax.ShapeDtypeStruct(A_k_cache.shape, dt),
        jax.ShapeDtypeStruct(A_v_cache.shape, dt),
        jax.ShapeDtypeStruct(A_wq.shape, dt),
        jax.ShapeDtypeStruct(A_wo.shape, dt),
        jax.ShapeDtypeStruct(B_w1.shape, dt),
        jax.ShapeDtypeStruct(B_w2.shape, dt),
    )
    scratch = [
        pltpu.VMEM((G, W, Dh), _BF16),
        pltpu.VMEM((G, W, Dh), _BF16),
        pltpu.VMEM(A_wq.shape, _BF16),
        pltpu.VMEM(A_wo.shape, _BF16),
        pltpu.VMEM(B_w1.shape, _BF16),
        pltpu.VMEM(B_w2.shape, _BF16),
        pltpu.VMEM(A_wq.shape, _BF16),
        pltpu.VMEM(A_wo.shape, _BF16),
        pltpu.VMEM(B_w1.shape, _BF16),
        pltpu.VMEM(B_w2.shape, _BF16),
        pltpu.VMEM((zrows, Dh), _BF16),
        pltpu.VMEM((G, 8, Dh), _F32),
        pltpu.VMEM((G, 8, Dh), _F32),
        pltpu.VMEM((G, 8, Dh), _F32),
        pltpu.VMEM((G, 8, W), _F32),
        pltpu.VMEM((B, Hq * Dh), _F32),
        pltpu.SemaphoreType.DMA((G,)),
        pltpu.SemaphoreType.DMA((G,)),
        pltpu.SemaphoreType.DMA((4,)),
        pltpu.SemaphoreType.DMA((1,)),
        pltpu.SemaphoreType.DMA((4,)),
    ]
    out, gx, db1, db2, dk, dv, dwq, dwo, dw1, dw2 = pl.pallas_call(
        kernel,
        out_shape=out_shape,
        in_specs=[vmem] * 4 + [hbm] * 6,
        out_specs=(vmem,) * 4 + (hbm,) * 6,
        scratch_shapes=scratch,
        compiler_params=pltpu.CompilerParams(vmem_limit_bytes=100 * 1024 * 1024),
    )(
        A_x.reshape(B, D), grad_out.reshape(B, D), B_b1.reshape(1, F), B_b2.reshape(1, D),
        A_k_cache, A_v_cache, A_wq, A_wo, B_w1, B_w2,
    )
    return (out.reshape(B, Sq, D), gx.reshape(B, Sq, D), dk, dv, dwq, dwo, dw1,
            db1.reshape(F), dw2, db2.reshape(D))
```

```python
import math

import jax
import jax.numpy as jnp
import jax.experimental.pallas as pl
import jax.experimental.pallas.tpu as pltpu

_F32 = jnp.float32
_BF16 = jnp.bfloat16
_EPS = 1e-5
_GELU_C = math.sqrt(2.0 / math.pi)
_GELU_A = 0.044715

_NT = (((1,), (1,)), ((), ()))
_TN = (((0,), (0,)), ((), ()))


def _dot(a, b):
    return jnp.dot(a, b, preferred_element_type=_F32)


def _dot_nt(a, b):
    return jax.lax.dot_general(a, b, _NT, preferred_element_type=_F32)


def _dot_tn(a, b):
    return jax.lax.dot_general(a, b, _TN, preferred_element_type=_F32)


def _ln_fwd(x):
    m = jnp.mean(x, axis=-1, keepdims=True)
    xc = x - m
    v = jnp.mean(xc * xc, axis=-1, keepdims=True)
    rstd = 1.0 / jnp.sqrt(v + _EPS)
    return xc * rstd, rstd


def _ln_bwd(dn, n, rstd):
    return (dn - jnp.mean(dn, axis=-1, keepdims=True)
            - n * jnp.mean(dn * n, axis=-1, keepdims=True)) * rstd


def _gelu_fwd(h):
    t = jnp.tanh(_GELU_C * (h + _GELU_A * h * h * h))
    return 0.5 * h * (1.0 + t), t


def _gelu_grad(h, t):
    return 0.5 * (1.0 + t) + 0.5 * h * (1.0 - t * t) * _GELU_C * (1.0 + 3.0 * _GELU_A * h * h)


def _scatter_plan(shape):
    rows, cols = shape
    nsplit = 1
    while rows % (2 * nsplit * 32) == 0 and (rows // (2 * nsplit)) * cols * 2 >= 448 * 1024:
        nsplit *= 2
    if cols <= 512:
        return nsplit, 32, cols
    for c in (1024, 896, 512, 256, 128):
        if cols % c == 0:
            return nsplit, 16, c
    return nsplit, 16, cols


def _make_kernel(B, D, Hq, Hkv, Sk, Dh, W, F, piece):
    rep = Hq // Hkv
    G = B * Hkv
    scale = Dh ** -0.5
    nz = Sk - W
    nblk = Sk // W
    assert 2 * rep == 8 and Sk % W == 0 and W % piece == 0

    def kernel(x_hbm, go_hbm, b1_hbm, b2_hbm,
               k_hbm, v_hbm, wq_hbm, wo_hbm, w1_hbm, w2_hbm,
               out_hbm, gx_hbm, dk_hbm, dv_hbm, dwq_hbm, dwo_hbm, dw1_hbm, db1_hbm,
               dw2_hbm, db2_hbm,
               x_v, go_v, b1_v, b2_v, out_v, gx_v, db1_v, db2_v,
               kbuf, vbuf, wq, wo, w1, w2, gwq, gwo, gw1, gw2, zbuf,
               q_scr, do_scr, a_scr, p_scr, flat_scr,
               rsem, zsem, osem):
        reads = [pltpu.make_async_copy(s, d, rsem.at[0]) for s, d in (
            (x_hbm, x_v), (go_hbm, go_v), (b1_hbm, b1_v), (b2_hbm, b2_v),
            (wq_hbm, wq),
            (k_hbm.at[:, :, pl.ds(nz, W), :], kbuf),
            (v_hbm.at[:, :, pl.ds(nz, W), :], vbuf),
            (wo_hbm, wo), (w1_hbm, w1), (w2_hbm, w2))]
        for c in reads:
            c.start()
        zbuf[...] = jnp.zeros(zbuf.shape, zbuf.dtype)
        q_scr[...] = jnp.zeros(q_scr.shape, _F32)
        do_scr[...] = jnp.zeros(do_scr.shape, _F32)
        for c in reads:
            c.wait()

        def zcopy(o_hbm, c):
            return pltpu.make_async_copy(
                zbuf, o_hbm.at[:, :, pl.ds(0, nblk - 1), pl.ds(c * piece, piece), :],
                zsem.at[0])

        def zstart(c, carry):
            zcopy(dk_hbm, c).start()
            zcopy(dv_hbm, c).start()
            return carry
        jax.lax.fori_loop(0, W // piece, zstart, 0)

        writes = []

        def write(src, dst):
            cp = pltpu.make_async_copy(src, dst, osem.at[0])
            cp.start()
            writes.append(cp)

        def write_grad(src, dst, val):
            ns, rows, cols = src.shape
            _, pr, pc = _scatter_plan((ns * rows, cols))
            src[...] = val.astype(_BF16).reshape(src.shape)
            for r in range(rows // pr):
                for c in range(cols // pc):
                    idx = (slice(None), pl.ds(r * pr, pr), pl.ds(c * pc, pc))
                    write(src.at[idx], dst.at[idx])

        def scatter_heads(dst, flat, layer):
            for b in range(B):
                for h in range(Hq):
                    dst[b * Hkv + h // rep, pl.ds(layer * rep + h % rep, 1), :] = (
                        flat[b:b + 1, h * Dh:(h + 1) * Dh])

        def gather_heads(src, layer):
            for b in range(B):
                for h in range(Hq):
                    flat_scr[pl.ds(b, 1), pl.ds(h * Dh, Dh)] = (
                        src[b * Hkv + h // rep, pl.ds(layer * rep + h % rep, 1), :])
            return flat_scr[...]

        def attn_fwd():
            def body(i, carry):
                b, g = i // Hkv, i % Hkv
                s = _dot_nt(q_scr[i].astype(_BF16), kbuf[b, g]) * scale
                m = jnp.max(s, axis=-1, keepdims=True)
                e = jnp.exp(s - m)
                p = e / jnp.sum(e, axis=-1, keepdims=True)
                p_scr[i] = p
                a_scr[i] = _dot(p.astype(_BF16), vbuf[b, g])
                return carry
            jax.lax.fori_loop(0, G, body, 0)

        def attn_bwd(last):
            def body(i, carry):
                b, g = i // Hkv, i % Hkv
                do = do_scr[i].astype(_BF16)
                p = p_scr[i]
                dp = _dot_nt(do, vbuf[b, g])
                ds = (p * (dp - jnp.sum(dp * p, axis=-1, keepdims=True)) * scale).astype(_BF16)
                a_scr[i] = _dot(ds, kbuf[b, g])
                if last:
                    kbuf[b, g] = _dot_tn(ds, q_scr[i].astype(_BF16)).astype(_BF16)
                    vbuf[b, g] = _dot_tn(p.astype(_BF16), do).astype(_BF16)
                return carry
            jax.lax.fori_loop(0, G, body, 0)

        b1 = b1_v[...].astype(_F32).reshape(1, F)
        b2 = b2_v[...].astype(_F32).reshape(1, D)

        x = x_v[...].astype(_F32)
        saved = []
        for layer in range(2):
            n_a, r_a = _ln_fwd(x)
            q = _dot(n_a.astype(_BF16), wq[...])
            scatter_heads(q_scr, q, layer)
            attn_fwd()
            o = gather_heads(a_scr, layer)
            x = x + _dot(o.astype(_BF16), wo[...])
            n_m, r_m = _ln_fwd(x)
            h = _dot(n_m.astype(_BF16), w1[...]) + b1
            g, t = _gelu_fwd(h)
            x = x + _dot(g.astype(_BF16), w2[...]) + b2
            saved.append((n_a, r_a, o, n_m, r_m, h, g, t))
        out_v[...] = x.astype(out_v.dtype)
        write(out_v, out_hbm)

        dx = go_v[...].astype(_F32)
        grads = [None, None]
        for layer in (1, 0):
            n_a, r_a, o, n_m, r_m, h, g, t = saved[layer]
            dm = dx
            dg = _dot_nt(dm.astype(_BF16), w2[...])
            dh = dg * _gelu_grad(h, t)
            dn = _dot_nt(dh.astype(_BF16), w1[...])
            dx = dx + _ln_bwd(dn, n_m, r_m)
            da = dx
            do = _dot_nt(da.astype(_BF16), wo[...])
            scatter_heads(do_scr, do, layer)
            attn_bwd(layer == 0)
            dq = gather_heads(a_scr, layer)
            dn = _dot_nt(dq.astype(_BF16), wq[...])
            dx = dx + _ln_bwd(dn, n_a, r_a)
            grads[layer] = (dm, dh, da, dq)
        for c in range(W // piece):
            for src, dst in ((kbuf, dk_hbm), (vbuf, dv_hbm)):
                write(src.at[:, :, pl.ds(c * piece, piece), :],
                      dst.at[:, :, nblk - 1, pl.ds(c * piece, piece), :])
        gx_v[...] = dx.astype(gx_v.dtype)
        write(gx_v, gx_hbm)

        def stack(a0, a1):
            return jnp.concatenate([a0, a1], axis=0).astype(_BF16)

        s0, s1 = saved
        g0, g1 = grads
        write_grad(gwq, dwq_hbm, _dot_tn(stack(s0[0], s1[0]), stack(g0[3], g1[3])))
        write_grad(gwo, dwo_hbm, _dot_tn(stack(s0[2], s1[2]), stack(g0[2], g1[2])))
        write_grad(gw1, dw1_hbm, _dot_tn(stack(s0[3], s1[3]), stack(g0[1], g1[1])))
        write_grad(gw2, dw2_hbm, _dot_tn(stack(s0[6], s1[6]), stack(g0[0], g1[0])))
        db1_v[...] = jnp.sum(g0[1] + g1[1], axis=0).astype(db1_v.dtype)
        write(db1_v, db1_hbm)
        db2_v[...] = jnp.sum(g0[0] + g1[0], axis=0).astype(db2_v.dtype)
        write(db2_v, db2_hbm)

        def zwait(c, carry):
            zcopy(dk_hbm, c).wait()
            zcopy(dv_hbm, c).wait()
            return carry
        jax.lax.fori_loop(0, W // piece, zwait, 0)
        for cp in writes:
            cp.wait()

    return kernel


@jax.jit
def pallas_interleave_layers__sliding_block_cached__dense_activation_gelu__decode_kernel(
    A_x: jax.Array,
    A_k_cache: jax.Array,
    A_v_cache: jax.Array,
    A_wq: jax.Array,
    A_wo: jax.Array,
    B_x: jax.Array,
    B_w1: jax.Array,
    B_b1: jax.Array,
    B_w2: jax.Array,
    B_b2: jax.Array,
    grad_out: jax.Array,
):
    B, Sq, D = A_x.shape
    assert Sq == 1
    Hq, Dh = 32, 128
    Hkv, Sk = A_k_cache.shape[1], A_k_cache.shape[2]
    W = min(4096, max(256, Sk // 4))
    F = B_w1.shape[1]
    G = B * Hkv
    piece = 128

    kernel = _make_kernel(B, D, Hq, Hkv, Sk, Dh, W, F, piece)

    hbm = pl.BlockSpec(memory_space=pl.ANY)
    like = lambda a: jax.ShapeDtypeStruct(a.shape, a.dtype)
    x2 = A_x.reshape(B, D)
    go2 = grad_out.reshape(B, D)
    dcache = jax.ShapeDtypeStruct((B, Hkv, Sk // W, W, Dh), A_k_cache.dtype)

    def split(a):
        ns = _scatter_plan(a.shape)[0]
        return jax.ShapeDtypeStruct((ns, a.shape[0] // ns, a.shape[1]), a.dtype)

    out_shape = (like(x2), like(x2), dcache, dcache, split(A_wq), split(A_wo),
                 split(B_w1), like(B_b1), split(B_w2), like(B_b2))
    vm = lambda a: pltpu.VMEM(a.shape, a.dtype)
    scratch = [
        vm(x2), vm(go2), vm(B_b1), vm(B_b2),
        vm(x2), vm(x2), vm(B_b1), vm(B_b2),
        pltpu.VMEM((B, Hkv, W, Dh), _BF16),
        pltpu.VMEM((B, Hkv, W, Dh), _BF16),
        vm(A_wq), vm(A_wo), vm(B_w1), vm(B_w2),
        vm(split(A_wq)), vm(split(A_wo)), vm(split(B_w1)), vm(split(B_w2)),
        pltpu.VMEM((B, Hkv, Sk // W - 1, piece, Dh), _BF16),
        pltpu.VMEM((G, 8, Dh), _F32),
        pltpu.VMEM((G, 8, Dh), _F32),
        pltpu.VMEM((G, 8, Dh), _F32),
        pltpu.VMEM((G, 8, W), _F32),
        pltpu.VMEM((B, Hq * Dh), _F32),
        pltpu.SemaphoreType.DMA((1,)),
        pltpu.SemaphoreType.DMA((1,)),
        pltpu.SemaphoreType.DMA((1,)),
    ]
    out, gx, dk, dv, dwq, dwo, dw1, db1, dw2, db2 = pl.pallas_call(
        kernel,
        out_shape=out_shape,
        in_specs=[hbm] * 10,
        out_specs=(hbm,) * 10,
        scratch_shapes=scratch,
        compiler_params=pltpu.CompilerParams(vmem_limit_bytes=100 * 1024 * 1024),
    )(x2, go2, B_b1, B_b2, A_k_cache, A_v_cache, A_wq, A_wo, B_w1, B_w2)
    return (out.reshape(A_x.shape), gx.reshape(A_x.shape),
            dk.reshape(A_k_cache.shape), dv.reshape(A_v_cache.shape),
            dwq.reshape(A_wq.shape), dwo.reshape(A_wo.shape), dw1.reshape(B_w1.shape),
            db1, dw2.reshape(B_w2.shape), db2)
```
